```python
import os as _os
_os.environ.setdefault("JAX_PLATFORMS", "cpu")
import jax
import jax.numpy as jnp

def _softmax(x, axis=-1):
    return jax.nn.softmax(x, axis=axis)
def _gelu(x):
    return jax.nn.gelu(x, approximate=True)
def _silu(x):
    return jax.nn.silu(x)
def _sigmoid(x):
    return jax.nn.sigmoid(x)
def _layernorm(x, axis=-1, eps=1e-5):
    m = jnp.mean(x, axis=axis, keepdims=True)
    v = jnp.var(x, axis=axis, keepdims=True)
    return (x - m) / jnp.sqrt(v + eps)
def _scatter_add(tgt, idx, src, axis=0):
    return tgt.at[idx].add(src)
def _segment_sum(src, seg, n):
    return jax.ops.segment_sum(src, seg, n)
class _Rng:
    def __init__(self, key):
        self._k = key
    def _next(self):
        self._k, sub = jax.random.split(self._k)
        return sub
    def normal(self, shape):
        return jax.random.normal(self._next(), shape, dtype=jnp.bfloat16)
    def randint(self, lo, hi, shape):
        return jax.random.randint(self._next(), shape, lo, hi, dtype=jnp.int32)
    def uniform(self, shape, lo=0.0, hi=1.0):
        return jax.random.uniform(self._next(), shape, jnp.bfloat16, lo, hi)
    def permutation(self, n):
        return jax.random.permutation(self._next(), n)


kernel_name = 'interleave_layers__gqa_block_cached__dense_activation_mish__decode'

def setup_inputs():
    _rng = _Rng(jax.random.key(int.from_bytes(__import__("os").urandom(4), "little")))
    _w = (lambda a: (lambda t: t.astype(jnp.bfloat16) if jnp.issubdtype(t.dtype, jnp.floating) else t)(jnp.asarray(a)))
    def _A_setup():
        B, Sq, D = 1, 1, 512
        Hq, Hkv, Sk, Dh = 32, 8, 65536, 128
        assert Hq % Hkv == 0, (Hq, Hkv)
        return {
            "x": _w((lambda *s: _rng.normal(s) * 0.05)(B, Sq, D)),
            "k_cache": _w((lambda *s: _rng.normal(s) * 1.6)(B, Hkv, Sk, Dh)),
            "v_cache": _w((lambda *s: _rng.normal(s) * 1.6)(B, Hkv, Sk, Dh)),
            "wq": _w((lambda *s: _rng.normal(s) * 1.6)(D, Hq * Dh) * (D ** -0.5)),
            "wo": _w((lambda *s: _rng.normal(s) * 1.6)(Hq * Dh, D) * ((Hq * Dh) ** -0.5)),
        }
    _A_in = _A_setup()

    def _B_setup():
        B, S, D, F = 1, 1, 512, 1792
        return {
            "x": _w((lambda *s: _rng.normal(s) * 0.05)(B, S, D)),
            "w1": _w((lambda *s: _rng.normal(s) * 0.8)(D, F) * (D ** -0.5)),
            "b1": _w((lambda *s: _rng.normal(s) * 0.8)(F)),
            "w2": _w((lambda *s: _rng.normal(s) * 0.8)(F, D) * (F ** -0.5)),
        }
    _B_in = _B_setup()

    return {
        "A_x": _A_in["x"],
        "A_k_cache": _A_in["k_cache"],
        "A_v_cache": _A_in["v_cache"],
        "A_wq": _A_in["wq"],
        "A_wo": _A_in["wo"],
        "B_x": _B_in["x"],
        "B_w1": _B_in["w1"],
        "B_b1": _B_in["b1"],
        "B_w2": _B_in["w2"],
    }

def reference(A_x, A_k_cache, A_v_cache, A_wq, A_wo, B_x, B_w1, B_b1, B_w2):
    def _A_ref(x, k_cache, v_cache, wq, wo):
        B, Sq, D = x.shape
        Hq, Dh = 32, 128
        Hkv = k_cache.shape[1]
        rep = Hq // Hkv
        q = (lambda x, *d: x.transpose(*d))((x @ wq).reshape(B, Sq, Hq, Dh), 0, 2, 1, 3)
        k = jnp.repeat(k_cache, rep, axis=1)
        v = jnp.repeat(v_cache, rep, axis=1)
        scores = jnp.einsum("bhqd,bhkd->bhqk", q, k) * (Dh ** -0.5)
        p = _softmax(scores, axis=-1)
        o = jnp.einsum("bhqk,bhkd->bhqd", p, v)
        return (lambda x, *d: x.transpose(*d))(o, 0, 2, 1, 3).reshape(B, Sq, Hq * Dh) @ wo

    def _B_ref(x, w1, b1, w2):
        h = jnp.einsum("bsd,df->bsf", x, w1) + b1
        sp = jnp.log1p(jnp.exp(-jnp.abs(h))) + jnp.where(h > 0, h, jnp.zeros_like(h))
        act = h * jnp.tanh(sp)
        return jnp.einsum("bsf,fd->bsd", act, w2)

    x = A_x
    x = x + _A_ref(_layernorm(x, axis=-1), A_k_cache, A_v_cache, A_wq, A_wo)
    x = x + _B_ref(_layernorm(x, axis=-1), B_w1, B_b1, B_w2)
    x = x + _A_ref(_layernorm(x, axis=-1), A_k_cache, A_v_cache, A_wq, A_wo)
    x = x + _B_ref(_layernorm(x, axis=-1), B_w1, B_b1, B_w2)
    return x
```

```python
import math

import jax
import jax.numpy as jnp
from jax import lax
import jax.experimental.pallas as pl
import jax.experimental.pallas.tpu as pltpu

_BS = 4096
_NSLOT = 58
_DEPTH = 6
_EPS = 1e-5


def _layernorm(x):
    m = jnp.mean(x, axis=-1, keepdims=True)
    d = x - m
    v = jnp.mean(d * d, axis=-1, keepdims=True)
    return d / jnp.sqrt(v + _EPS)


@jax.jit
def pallas_interleave_layers__gqa_block_cached__dense_activation_mish__decode_kernel(
    A_x: jax.Array,
    A_k_cache: jax.Array,
    A_v_cache: jax.Array,
    A_wq: jax.Array,
    A_wo: jax.Array,
    B_x: jax.Array,
    B_w1: jax.Array,
    B_b1: jax.Array,
    B_w2: jax.Array,
):
    del B_x
    _, _, D = A_x.shape
    _, Hkv, S, Dh = A_k_cache.shape
    Hq = A_wq.shape[1] // Dh
    G = Hq // Hkv
    GD = G * Dh
    F = B_w1.shape[1]
    BS, N, DEPTH = _BS, _NSLOT, _DEPTH
    CPH = S // BS
    C = Hkv * CPH
    QR = 8
    qk_scale = (Dh ** -0.5) * math.log2(math.e)
    bf16, f32 = jnp.bfloat16, jnp.float32

    def kernel(x_hbm, k_hbm, v_hbm, wq_hbm, wo_hbm, w1_hbm, b1_hbm, w2_hbm, o_ref,
               kbuf, vbuf, wq, wo, w1, w2, xb, b1b, ksem, vsem, wsem):

        def kv_copies(c):
            slot = c % N
            h = c // CPH
            r = pl.multiple_of((c % CPH) * BS, BS)
            return (pltpu.make_async_copy(k_hbm.at[0, h, pl.ds(r, BS)], kbuf.at[slot], ksem.at[slot]),
                    pltpu.make_async_copy(v_hbm.at[0, h, pl.ds(r, BS)], vbuf.at[slot], vsem.at[slot]))

        def kv_start(c):
            a, b = kv_copies(c)
            a.start()
            b.start()

        def w_copies():
            cps = []
            for h in range(Hkv):
                cps.append(pltpu.make_async_copy(wq_hbm.at[:, pl.ds(h * GD, GD)], wq.at[h], wsem.at[h]))
            for h in range(Hkv):
                cps.append(pltpu.make_async_copy(wo_hbm.at[pl.ds(h * GD, GD), :], wo.at[h], wsem.at[Hkv + h]))
            cps.append(pltpu.make_async_copy(w1_hbm, w1, wsem.at[2 * Hkv]))
            cps.append(pltpu.make_async_copy(w2_hbm, w2, wsem.at[2 * Hkv + 1]))
            cps.append(pltpu.make_async_copy(b1_hbm, b1b, wsem.at[2 * Hkv + 2]))
            cps.append(pltpu.make_async_copy(x_hbm, xb, wsem.at[2 * Hkv + 3]))
            return cps

        cps = w_copies()
        x_cp = cps[-1]
        x_cp.start()
        cps[0].start()
        kv_start(0)
        for cp in cps[1:-1]:
            cp.start()
        for c in range(1, DEPTH):
            kv_start(c)

        row = lax.broadcasted_iota(jnp.int32, (QR, Dh), 0)

        def attention(xn, layer):
            xn8 = jnp.broadcast_to(xn, (QR, D)).astype(bf16)

            def head_body(hi, out_acc):
                h = hi if layer == 0 else Hkv - 1 - hi
                if layer == 0:
                    pltpu.make_async_copy(wq_hbm.at[:, pl.ds(0, GD)], wq.at[h], wsem.at[h]).wait()
                qf = jnp.dot(xn8, wq[h], preferred_element_type=f32)
                q = qf[:, 0:Dh]
                for g in range(1, G):
                    q = jnp.where(row == g, qf[:, g * Dh:(g + 1) * Dh], q)
                qb = q.astype(bf16)

                def chunk_body(ji, carry):
                    m, l, acc = carry
                    j = ji if layer == 0 else CPH - 1 - ji
                    c = h * CPH + j
                    slot = c % N
                    kc, vc = kv_copies(c)
                    if layer == 0:
                        kc.wait()
                    else:
                        @pl.when(c < C - N)
                        def _():
                            kc.wait()
                            vc.wait()
                    s = lax.dot_general(qb, kbuf[slot], (((1,), (1,)), ((), ())), preferred_element_type=f32)
                    s = s * qk_scale
                    m_new = jnp.maximum(m, jnp.max(s, axis=1, keepdims=True))
                    alpha = jnp.exp2(m - m_new)
                    p = jnp.exp2(s - m_new)
                    l = alpha * l + jnp.sum(p, axis=1, keepdims=True)
                    if layer == 0:
                        vc.wait()
                    acc = alpha * acc + jnp.dot(p.astype(bf16), vbuf[slot], preferred_element_type=f32)
                    if layer == 0:
                        @pl.when(c + DEPTH < C)
                        def _():
                            kv_start(c + DEPTH)
                    else:
                        @pl.when(c - N >= 0)
                        def _():
                            kv_start(c - N)
                    return m_new, l, acc

                m0 = jnp.full((QR, 1), -jnp.inf, f32)
                l0 = jnp.zeros((QR, 1), f32)
                a0 = jnp.zeros((QR, Dh), f32)
                _, l, acc = lax.fori_loop(0, CPH, chunk_body, (m0, l0, a0))
                o = (acc / l).astype(bf16)
                zero = jnp.zeros_like(o)
                od = jnp.concatenate([jnp.where(row == g, o, zero) for g in range(G)], axis=1)
                if layer == 0:
                    pltpu.make_async_copy(wo_hbm.at[pl.ds(0, GD), :], wo.at[h], wsem.at[Hkv + h]).wait()
                return out_acc + jnp.dot(od, wo[h], preferred_element_type=f32)

            out = lax.fori_loop(0, Hkv, head_body, jnp.zeros((QR, D), f32))
            return jnp.sum(out, axis=0, keepdims=True)

        def mlp(xn):
            xn8 = jnp.broadcast_to(xn, (QR, D)).astype(bf16)
            hmid = jnp.dot(xn8, w1[...], preferred_element_type=f32) + b1b[...].astype(f32).reshape(1, F)
            sp = jnp.log1p(jnp.exp(-jnp.abs(hmid))) + jnp.maximum(hmid, 0.0)
            act = hmid * jnp.tanh(sp)
            y = jnp.dot(act.astype(bf16), w2[...], preferred_element_type=f32)
            return y[0:1, :]

        def rnd(t):
            return t.astype(bf16).astype(f32)

        x_cp.wait()
        x = xb[0].astype(f32)
        for layer in range(2):
            x = rnd(x + rnd(attention(_layernorm(x), layer)))
            if layer == 0:
                for cp in cps[-4:-1]:
                    cp.wait()
            x = rnd(x + rnd(mlp(_layernorm(x))))
        o_ref[0] = x.astype(o_ref.dtype)

    hbm = pl.BlockSpec(memory_space=pl.ANY)
    return pl.pallas_call(
        kernel,
        out_shape=jax.ShapeDtypeStruct(A_x.shape, A_x.dtype),
        in_specs=[hbm] * 8,
        out_specs=pl.BlockSpec(memory_space=pltpu.VMEM),
        scratch_shapes=[
            pltpu.VMEM((N, BS, Dh), bf16),
            pltpu.VMEM((N, BS, Dh), bf16),
            pltpu.VMEM((Hkv, D, GD), bf16),
            pltpu.VMEM((Hkv, GD, D), bf16),
            pltpu.VMEM((D, F), bf16),
            pltpu.VMEM((F, D), bf16),
            pltpu.VMEM(A_x.shape, bf16),
            pltpu.VMEM((F,), bf16),
            pltpu.SemaphoreType.DMA((N,)),
            pltpu.SemaphoreType.DMA((N,)),
            pltpu.SemaphoreType.DMA((2 * Hkv + 4,)),
        ],
        compiler_params=pltpu.CompilerParams(vmem_limit_bytes=128 * 1024 * 1024),
    )(A_x, A_k_cache, A_v_cache, A_wq, A_wo, B_w1, B_b1, B_w2)
```

```python
import math

import numpy as np
import jax
import jax.numpy as jnp
from jax import lax
import jax.experimental.pallas as pl
import jax.experimental.pallas.tpu as pltpu

_BS = 4096
_NSTAGE = 2
_NPACK = 69
_EPS = 1e-5


def _c32(v):
    return np.uint32(v).astype(np.int32)


_M_E = _c32(0x7F807F80)
_M_SM = _c32(0x807F807F)
_M_M = _c32(0x007F007F)
_M_M7 = _c32(0x3F803F80)
_M_S14 = _c32(0x40004000)
_M_S15 = _c32(0x80008000)
_M_D7 = _c32(0x0F800F80)
_M_BAD = _c32(0xF000F000)


def _lsr(x, n):
    return lax.shift_right_logical(x, jnp.int32(n))


def _lsl(x, n):
    return lax.shift_left(x, jnp.int32(n))


def _encode(W, base7):
    out = []
    for j in range(8):
        a, b = W[2 * j], W[2 * j + 1]
        out.append((a & _M_SM) | (_lsl(b, 7) & _M_M7) | (_lsr(b, 1) & _M_S14))
    t = [(w & _M_E) - base7 for w in W]
    bad = t[0]
    for w in t[1:]:
        bad = bad | w
    for i in range(5):
        out.append(_lsr(t[3 * i], 7) | _lsr(t[3 * i + 1], 2) | _lsl(t[3 * i + 2], 3)
                   | (_lsl(t[15], 8 - i) & _M_S15))
    return out, bad


def _decode(P, base7):
    S, E = P[:8], P[8:]
    W = [None] * 16
    for j in range(8):
        W[2 * j] = S[j] & _M_SM
        W[2 * j + 1] = (_lsr(S[j], 7) & _M_M) | (_lsl(S[j], 1) & _M_S15)
    for i in range(5):
        W[3 * i] = W[3 * i] | ((_lsl(E[i], 7) & _M_D7) + base7)
        W[3 * i + 1] = W[3 * i + 1] | ((_lsl(E[i], 2) & _M_D7) + base7)
        W[3 * i + 2] = W[3 * i + 2] | ((_lsr(E[i], 3) & _M_D7) + base7)
    d = None
    for i in range(5):
        b = _lsr(E[i], 8 - i) & _c32(0x00800080 << i)
        d = b if d is None else d | b
    W[15] = W[15] | (d + base7)
    return W


def _layernorm(x):
    m = jnp.mean(x, axis=-1, keepdims=True)
    d = x - m
    v = jnp.mean(d * d, axis=-1, keepdims=True)
    return d / jnp.sqrt(v + _EPS)


@jax.jit
def pallas_interleave_layers__gqa_block_cached__dense_activation_mish__decode_kernel(
    A_x: jax.Array,
    A_k_cache: jax.Array,
    A_v_cache: jax.Array,
    A_wq: jax.Array,
    A_wo: jax.Array,
    B_x: jax.Array,
    B_w1: jax.Array,
    B_b1: jax.Array,
    B_w2: jax.Array,
):
    del B_x
    _, _, D = A_x.shape
    _, Hkv, S, Dh = A_k_cache.shape
    Hq = A_wq.shape[1] // Dh
    G = Hq // Hkv
    GD = G * Dh
    F = B_w1.shape[1]
    BS, NST, Z = _BS, _NSTAGE, _NPACK
    RW = BS // 2
    NG = RW // 128
    PW = NG * 104
    UPH = S // BS
    C = Hkv * UPH
    NS = C - NST - Z
    SB = Z * 2 * PW
    ROWS = SB + NST * 2 * RW
    assert C % NST == 0 and NS >= NST and (NS - NST) * 16 <= Z * 13
    QR = 8
    qk_scale = (Dh ** -0.5) * math.log2(math.e)
    bf16, f32, i32 = jnp.bfloat16, jnp.float32, jnp.int32

    def kernel(x_hbm, k_hbm, v_hbm, wq_hbm, wo_hbm, w1_hbm, b1_hbm, w2_hbm, o_ref,
               arena, wq, wo, w1, w2, xb, b1b, st, meta, ksem, vsem, wsem, fsem):
        k32 = k_hbm.bitcast(i32)
        v32 = v_hbm.bitcast(i32)

        def kv_copies(c, row, si):
            h = c // UPH
            r = pl.multiple_of((c % UPH) * RW, RW)
            row = pl.multiple_of(row, 8)
            return (pltpu.make_async_copy(k32.at[0, h, pl.ds(r, RW)], arena.at[pl.ds(row, RW)], ksem.at[si]),
                    pltpu.make_async_copy(v32.at[0, h, pl.ds(r, RW)], arena.at[pl.ds(row + RW, RW)], vsem.at[si]))

        def stage_copies(c):
            s = c % NST
            return kv_copies(c, SB + s * 2 * RW, s)

        def land_row(i):
            return jnp.where(i < NST, SB + (NST - 1 - i) * 2 * RW, (i - NST) * 2 * RW)

        def stream_copies(i):
            return kv_copies(NS - 1 - i, land_row(i), i)

        def start(cps):
            for cp in cps:
                cp.start()

        def w_copies():
            cps = []
            for h in range(Hkv):
                cps.append(pltpu.make_async_copy(wq_hbm.at[:, pl.ds(h * GD, GD)], wq.at[h], wsem.at[h]))
            for h in range(Hkv):
                cps.append(pltpu.make_async_copy(wo_hbm.at[pl.ds(h * GD, GD), :], wo.at[h], wsem.at[Hkv + h]))
            cps.append(pltpu.make_async_copy(w1_hbm, w1, wsem.at[2 * Hkv]))
            cps.append(pltpu.make_async_copy(w2_hbm, w2, wsem.at[2 * Hkv + 1]))
            cps.append(pltpu.make_async_copy(b1_hbm, b1b, wsem.at[2 * Hkv + 2]))
            cps.append(pltpu.make_async_copy(x_hbm, xb, wsem.at[2 * Hkv + 3]))
            return cps

        cps = w_copies()
        x_cp = cps[-1]
        x_cp.start()
        cps[0].start()
        start(stage_copies(0))
        start(cps[1:-1])
        for c in range(1, NST):
            start(stage_copies(c))

        row = lax.broadcasted_iota(i32, (QR, Dh), 0)

        def raw_rows(r0):
            return pltpu.bitcast(arena[pl.ds(pl.multiple_of(r0, 8), RW), :], bf16)

        def unpack_rows(p0, base):
            p0 = pl.multiple_of(p0, 8)
            base7 = jnp.full((8, Dh), base * (128 * 65537), i32)
            words = []
            for g in range(NG):
                P = [arena[pl.ds(p0 + (g * 13 + i) * 8, 8), :] for i in range(13)]
                words += _decode(P, base7)
            return pltpu.bitcast(jnp.concatenate(words, axis=0), bf16)

        def pack_rows(r0, p0):
            r0 = pl.multiple_of(r0, 8)
            p0 = pl.multiple_of(p0, 8)
            head = arena[pl.ds(r0, 128), :]
            ex = jnp.maximum(head & _c32(0x7F800000), _lsl(head, 16) & _c32(0x7F800000))
            emax = _lsr(jnp.max(ex), 23)
            base = jnp.clip(emax + 2 - 31, 0, 224)
            base7 = jnp.full((8, Dh), base * (128 * 65537), i32)
            bad = jnp.zeros((8, Dh), i32)
            for g in range(NG):
                W = [arena[pl.ds(r0 + (g * 16 + i) * 8, 8), :] for i in range(16)]
                P, b = _encode(W, base7)
                bad = bad | b
                for i in range(13):
                    arena[pl.ds(p0 + (g * 13 + i) * 8, 8), :] = P[i]
            return base, bad

        def softmax_step(qb, kmat):
            s = lax.dot_general(qb, kmat, (((1,), (1,)), ((), ())), preferred_element_type=f32)
            s = s * qk_scale
            m = st[0]
            m_new = jnp.maximum(m, jnp.max(s, axis=1, keepdims=True))
            alpha = jnp.exp2(m - m_new)
            p = jnp.exp2(s - m_new[:, 0:1])
            st[0] = m_new
            st[1] = alpha * st[1] + jnp.sum(p, axis=1, keepdims=True)
            return alpha, p.astype(bf16)

        def pv_step(alpha, pb, vmat):
            st[2] = alpha * st[2] + jnp.dot(pb, vmat, preferred_element_type=f32)

        def attention(xn, layer):
            xn8 = jnp.broadcast_to(xn, (QR, D)).astype(bf16)

            def head_body(hi, out_acc):
                h = hi if layer == 0 else Hkv - 1 - hi
                if layer == 0:
                    pltpu.make_async_copy(wq_hbm.at[:, pl.ds(0, GD)], wq.at[h], wsem.at[h]).wait()
                qf = jnp.dot(xn8, wq[h], preferred_element_type=f32)
                q = qf[:, 0:Dh]
                for g in range(1, G):
                    q = jnp.where(row == g, qf[:, g * Dh:(g + 1) * Dh], q)
                qb = q.astype(bf16)
                st[0] = jnp.full((QR, Dh), -jnp.inf, f32)
                st[1] = jnp.zeros((QR, Dh), f32)
                st[2] = jnp.zeros((QR, Dh), f32)

                def unit_first(ji, carry):
                    c = h * UPH + ji
                    r0 = SB + (c % NST) * 2 * RW
                    kc, vc = stage_copies(c)
                    kc.wait()
                    alpha, pb = softmax_step(qb, raw_rows(r0))
                    vc.wait()
                    pv_step(alpha, pb, raw_rows(r0 + RW))

                    @pl.when((c >= NS) & (c < C - NST))
                    def _():
                        z = C - NST - 1 - c
                        kbase, kbad = pack_rows(r0, z * 2 * PW)
                        vbase, vbad = pack_rows(r0 + RW, z * 2 * PW + PW)
                        meta[0, z] = kbase
                        meta[1, z] = vbase
                        meta[2, z] = jnp.max(jnp.where(((kbad | vbad) & _M_BAD) != 0, 1, 0))

                    @pl.when(c + NST < C)
                    def _():
                        start(stage_copies(c + NST))
                    return carry

                def unit_second(ji, carry):
                    c = h * UPH + (UPH - 1 - ji)
                    packed = (c >= NS) & (c < C - NST)
                    z = jnp.clip(C - NST - 1 - c, 0, Z - 1)
                    lossless = meta[2, z] == 0

                    @pl.when(jnp.logical_not(packed))
                    def _():
                        i = NS - 1 - c
                        streamed = c < NS
                        r0 = jnp.where(streamed, land_row(i), SB + (c % NST) * 2 * RW)
                        kc, vc = stream_copies(jnp.maximum(i, 0))

                        @pl.when(streamed)
                        def _():
                            kc.wait()
                        alpha, pb = softmax_step(qb, raw_rows(r0))

                        @pl.when(streamed)
                        def _():
                            vc.wait()
                        pv_step(alpha, pb, raw_rows(r0 + RW))

                        @pl.when(jnp.logical_not(streamed))
                        def _():
                            start(stream_copies(C - 1 - c))

                    @pl.when(packed & lossless)
                    def _():
                        alpha, pb = softmax_step(qb, unpack_rows(z * 2 * PW, meta[0, z]))
                        pv_step(alpha, pb, unpack_rows(z * 2 * PW + PW, meta[1, z]))

                    @pl.when(packed & jnp.logical_not(lossless))
                    def _():
                        r = pl.multiple_of((c % UPH) * RW, RW)
                        zone = arena.at[pl.ds(pl.multiple_of(z * 2 * PW, 8), RW)]
                        kc = pltpu.make_async_copy(k32.at[0, h, pl.ds(r, RW)], zone, fsem.at[0])
                        kc.start()
                        kc.wait()
                        alpha, pb = softmax_step(qb, raw_rows(z * 2 * PW))
                        vc = pltpu.make_async_copy(v32.at[0, h, pl.ds(r, RW)], zone, fsem.at[0])
                        vc.start()
                        vc.wait()
                        pv_step(alpha, pb, raw_rows(z * 2 * PW))

                    @pl.when(packed)
                    def _():
                        n_old = (z * 13) // 16
                        n_new = ((z + 1) * 13) // 16
                        i = NST + n_new - 1

                        @pl.when((n_new > n_old) & (i < NS))
                        def _():
                            start(stream_copies(i))
                    return carry

                lax.fori_loop(0, UPH, unit_first if layer == 0 else unit_second, 0)
                o = (st[2] / jnp.sum(st[1], axis=1, keepdims=True) * float(Dh)).astype(bf16) if False else \
                    (st[2] / st[1]).astype(bf16)
                zero = jnp.zeros_like(o)
                od = jnp.concatenate([jnp.where(row == g, o, zero) for g in range(G)], axis=1)
                if layer == 0:
                    pltpu.make_async_copy(wo_hbm.at[pl.ds(0, GD), :], wo.at[h], wsem.at[Hkv + h]).wait()
                return out_acc + jnp.dot(od, wo[h], preferred_element_type=f32)

            out = lax.fori_loop(0, Hkv, head_body, jnp.zeros((QR, D), f32))
            return jnp.sum(out, axis=0, keepdims=True)

        def mlp(xn):
            xn8 = jnp.broadcast_to(xn, (QR, D)).astype(bf16)
            hmid = jnp.dot(xn8, w1[...], preferred_element_type=f32) + b1b[...].astype(f32).reshape(1, F)
            sp = jnp.log1p(jnp.exp(-jnp.abs(hmid))) + jnp.maximum(hmid, 0.0)
            act = hmid * jnp.tanh(sp)
            y = jnp.dot(act.astype(bf16), w2[...], preferred_element_type=f32)
            return y[0:1, :]

        def rnd(t):
            return t.astype(bf16).astype(f32)

        x_cp.wait()
        x = xb[0].astype(f32)
        for layer in range(2):
            x = rnd(x + rnd(attention(_layernorm(x), layer)))
            if layer == 0:
                for cp in cps[-4:-1]:
                    cp.wait()
            x = rnd(x + rnd(mlp(_layernorm(x))))
        o_ref[0] = x.astype(o_ref.dtype)

    hbm = pl.BlockSpec(memory_space=pl.ANY)
    return pl.pallas_call(
        kernel,
        out_shape=jax.ShapeDtypeStruct(A_x.shape, A_x.dtype),
        in_specs=[hbm] * 8,
        out_specs=pl.BlockSpec(memory_space=pltpu.VMEM),
        scratch_shapes=[
            pltpu.VMEM((ROWS, Dh), i32),
            pltpu.VMEM((Hkv, D, GD), bf16),
            pltpu.VMEM((Hkv, GD, D), bf16),
            pltpu.VMEM((D, F), bf16),
            pltpu.VMEM((F, D), bf16),
            pltpu.VMEM(A_x.shape, bf16),
            pltpu.VMEM((F,), bf16),
            pltpu.VMEM((3, QR, Dh), f32),
            pltpu.SMEM((3, Z), i32),
            pltpu.SemaphoreType.DMA((NS,)),
            pltpu.SemaphoreType.DMA((NS,)),
            pltpu.SemaphoreType.DMA((2 * Hkv + 4,)),
            pltpu.SemaphoreType.DMA((1,)),
        ],
        compiler_params=pltpu.CompilerParams(vmem_limit_bytes=128 * 1024 * 1024),
    )(A_x, A_k_cache, A_v_cache, A_wq, A_wo, B_w1, B_b1, B_w2)
```

```python
import math

import numpy as np
import jax
import jax.numpy as jnp
from jax import lax
import jax.experimental.pallas as pl
import jax.experimental.pallas.tpu as pltpu

_BS = 4096
_NSTAGE = 2
_PACK_ROWS = 243968
_FORCE = None
_EPS = 1e-5


def _c32(v):
    return np.uint32(v).astype(np.int32)


_M_E = _c32(0x7F807F80)
_M_SM = _c32(0x807F807F)
_M_M = _c32(0x007F007F)
_M_M7 = _c32(0x3F803F80)
_M_S14 = _c32(0x40004000)
_M_S15 = _c32(0x80008000)
_M_D = {4: _c32(0x07800780), 5: _c32(0x0F800F80)}
_M_BAD = {4: _c32(0xF800F800), 5: _c32(0xF000F000)}


def _lsr(x, n):
    return lax.shift_right_logical(x, jnp.int32(n))


def _lsl(x, n):
    return lax.shift_left(x, jnp.int32(n))


def _encode(W, base7, nb):
    out = []
    for j in range(8):
        a, b = W[2 * j], W[2 * j + 1]
        out.append((a & _M_SM) | (_lsl(b, 7) & _M_M7) | (_lsr(b, 1) & _M_S14))
    t = [(w & _M_E) - base7 for w in W]
    bad = t[0]
    for w in t[1:]:
        bad = bad | w
    if nb == 5:
        for i in range(5):
            out.append(_lsr(t[3 * i], 7) | _lsr(t[3 * i + 1], 2) | _lsl(t[3 * i + 2], 3)
                       | (_lsl(t[15], 8 - i) & _M_S15))
    else:
        for i in range(4):
            out.append(_lsr(t[4 * i], 7) | _lsr(t[4 * i + 1], 3) | _lsl(t[4 * i + 2], 1) | _lsl(t[4 * i + 3], 5))
    return out, bad


def _decode(P, base7, nb):
    S, E = P[:8], P[8:]
    W = [None] * 16
    for j in range(8):
        W[2 * j] = S[j] & _M_SM
        W[2 * j + 1] = (_lsr(S[j], 7) & _M_M) | (_lsl(S[j], 1) & _M_S15)
    m = _M_D[nb]
    if nb == 5:
        for i in range(5):
            W[3 * i] = W[3 * i] | ((_lsl(E[i], 7) & m) + base7)
            W[3 * i + 1] = W[3 * i + 1] | ((_lsl(E[i], 2) & m) + base7)
            W[3 * i + 2] = W[3 * i + 2] | ((_lsr(E[i], 3) & m) + base7)
        d = None
        for i in range(5):
            b = _lsr(E[i], 8 - i) & _c32(0x00800080 << i)
            d = b if d is None else d | b
        W[15] = W[15] | (d + base7)
    else:
        for i in range(4):
            W[4 * i] = W[4 * i] | ((_lsl(E[i], 7) & m) + base7)
            W[4 * i + 1] = W[4 * i + 1] | ((_lsl(E[i], 3) & m) + base7)
            W[4 * i + 2] = W[4 * i + 2] | ((_lsr(E[i], 1) & m) + base7)
            W[4 * i + 3] = W[4 * i + 3] | ((_lsr(E[i], 5) & m) + base7)
    return W


def _exp_fields(w):
    hi = pltpu.bitcast(w & _c32(0x7F800000), jnp.float32)
    lo = pltpu.bitcast(_lsl(w, 16) & _c32(0x7F800000), jnp.float32)
    return hi, lo


def _layernorm(x):
    m = jnp.mean(x, axis=-1, keepdims=True)
    d = x - m
    v = jnp.mean(d * d, axis=-1, keepdims=True)
    return d / jnp.sqrt(v + _EPS)


@jax.jit
def pallas_interleave_layers__gqa_block_cached__dense_activation_mish__decode_kernel(
    A_x: jax.Array,
    A_k_cache: jax.Array,
    A_v_cache: jax.Array,
    A_wq: jax.Array,
    A_wo: jax.Array,
    B_x: jax.Array,
    B_w1: jax.Array,
    B_b1: jax.Array,
    B_w2: jax.Array,
):
    del B_x
    _, _, D = A_x.shape
    _, Hkv, S, Dh = A_k_cache.shape
    Hq = A_wq.shape[1] // Dh
    G = Hq // Hkv
    GD = G * Dh
    F = B_w1.shape[1]
    BS, NST = _BS, _NSTAGE
    RW = BS // 2
    NG = RW // 128
    PWS = {nb: NG * 8 * (8 + nb) for nb in (4, 5)}
    UPH = S // BS
    C = Hkv * UPH
    SB = _PACK_ROWS
    HW = D // 2
    WB = SB + NST * 2 * RW
    ROWS = WB + 2 * G * HW
    NW = Hkv - 1
    ZS = {nb: SB // (2 * PWS[nb]) for nb in (4, 5)}
    NSS = {nb: C - NST - ZS[nb] for nb in (4, 5)}
    ZMAX, NSMAX, NSMIN = max(ZS.values()), max(NSS.values()), min(NSS.values())
    for nb in (4, 5):
        assert NSS[nb] >= NST and (NW + 2 * NSS[nb] - 2 * NST) * RW <= ZS[nb] * 2 * PWS[nb]
        assert ZS[nb] * 2 * PWS[nb] + G * HW <= SB
    assert 2 * G * HW == RW and GD == D
    assert C % NST == 0
    QR = 8
    qk_scale = (Dh ** -0.5) * math.log2(math.e)
    bf16, f32, i32 = jnp.bfloat16, jnp.float32, jnp.int32

    def kernel(x_hbm, k_hbm, v_hbm, wq_hbm, wo_hbm, w1_hbm, b1_hbm, w2_hbm, o_ref,
               arena, w1, w2, xb, b1b, st, meta, cfg, ksem, vsem, hsem, wsem, fsem):
        k32 = k_hbm.bitcast(i32)
        v32 = v_hbm.bitcast(i32)
        wq32 = wq_hbm.bitcast(i32)
        wo32 = wo_hbm.bitcast(i32)

        def kv_copies(c, row, si):
            h = c // UPH
            r = pl.multiple_of((c % UPH) * RW, RW)
            row = pl.multiple_of(row, 8)
            return (pltpu.make_async_copy(k32.at[0, h, pl.ds(r, RW)], arena.at[pl.ds(row, RW)], ksem.at[si]),
                    pltpu.make_async_copy(v32.at[0, h, pl.ds(r, RW)], arena.at[pl.ds(row + RW, RW)], vsem.at[si]))

        def stage_copies(c):
            s = c % NST
            return kv_copies(c, SB + s * 2 * RW, s)

        def slot_row(s):
            stage = SB + ((NST - 1 - s // 2) * 2 + s % 2) * RW
            return jnp.where(s < 2 * NST, stage, (s - 2 * NST) * RW)

        def slots_free(e):
            pw = jnp.where(cfg[0] == 4, PWS[4], PWS[5])
            return jnp.minimum(e, 2 * NST) + (jnp.maximum(e - 2 * NST, 0) * pw) // RW

        def half_copy(j, ns, src):
            c = ns - 1 - j // 2
            h = c // UPH
            r = pl.multiple_of((c % UPH) * RW, RW)
            row = pl.multiple_of(slot_row(NW + j), 8)
            sem = (ksem if src is k32 else vsem).at[j // 2]
            return pltpu.make_async_copy(src.at[0, h, pl.ds(r, RW)], arena.at[pl.ds(row, RW)], sem)

        def head_w_row(h, layer, is_o):
            if layer == 0:
                r = (h % 2) * RW
            else:
                r = slot_row(NW - 1 - h)
            r = r + is_o * G * HW
            if layer == 1 and not is_o:
                spare = jnp.where(cfg[0] == 4, ZS[4] * 2 * PWS[4], ZS[5] * 2 * PWS[5])
                r = jnp.where(h == NW - 1, spare, r)
            return jnp.where(h == NW, WB + is_o * G * HW, r)

        def head_w_copies(h, layer, is_o):
            row = pl.multiple_of(head_w_row(h, layer, is_o), 8)
            cps = []
            for g in range(G):
                if is_o:
                    src = wo32.at[pl.ds(pl.multiple_of(h * G * Dh // 2, HW), HW), pl.ds(g * Dh, Dh)]
                else:
                    src = wq32.at[:, pl.ds(pl.multiple_of(h * GD + g * Dh, Dh), Dh)]
                cps.append(pltpu.make_async_copy(src, arena.at[pl.ds(row + g * HW, HW)], hsem.at[is_o, h]))
            return cps

        def head_w(h, layer, is_o, g):
            row = pl.multiple_of(head_w_row(h, layer, is_o) + g * HW, 8)
            return pltpu.bitcast(arena[pl.ds(row, HW), :], bf16)

        def refill(e, ns):
            s = slots_free(e) - 1
            fresh = s >= slots_free(e - 1)
            j = s - NW

            @pl.when(fresh & (s < NW))
            def _():
                @pl.when(s > 0)
                def _():
                    start(head_w_copies(NW - 1 - s, 1, 0))
                start(head_w_copies(NW - 1 - s, 1, 1))

            @pl.when(fresh & (j >= 0) & (j < 2 * ns))
            def _():
                @pl.when(j % 2 == 0)
                def _():
                    half_copy(j, ns, k32).start()

                @pl.when(j % 2 == 1)
                def _():
                    half_copy(j, ns, v32).start()

        def start(cps):
            for cp in cps:
                cp.start()

        def wait(cps):
            for cp in cps:
                cp.wait()

        x_cp = pltpu.make_async_copy(x_hbm, xb, wsem.at[0])
        w1_cp = pltpu.make_async_copy(w1_hbm, w1, wsem.at[1])
        b1_cp = pltpu.make_async_copy(b1_hbm, b1b, wsem.at[2])
        w2_cp = pltpu.make_async_copy(w2_hbm, w2, wsem.at[3])
        x_cp.start()
        start(head_w_copies(0, 0, 0))
        for c in range(NST):
            start(stage_copies(c))
        start(head_w_copies(0, 0, 1))
        for is_o in (0, 1):
            start(head_w_copies(1, 0, is_o))
            start(head_w_copies(NW, 0, is_o))
        w1_cp.start()
        b1_cp.start()

        cfg[0] = 5
        st[3] = jnp.zeros((QR, Dh), f32)
        st[4] = jnp.full((QR, Dh), jnp.inf, f32)
        row = lax.broadcasted_iota(i32, (QR, Dh), 0)

        def by_format(fn):
            for nb in (4, 5):
                pl.when(cfg[0] == nb)(lambda nb=nb: fn(nb))

        def n_streamed():
            return jnp.where(cfg[0] == 4, NSS[4], NSS[5])

        def raw_rows(r0):
            return pltpu.bitcast(arena[pl.ds(pl.multiple_of(r0, 8), RW), :], bf16)

        def unpack_rows(p0, base, nb):
            p0 = pl.multiple_of(p0, 8)
            base7 = jnp.full((8, Dh), base * (128 * 65537), i32)
            words = []
            for g in range(NG):
                P = [arena[pl.ds(p0 + (g * (8 + nb) + i) * 8, 8), :] for i in range(8 + nb)]
                words += _decode(P, base7, nb)
            return pltpu.bitcast(jnp.concatenate(words, axis=0), bf16)

        def sample_emax(r0):
            hi, lo = _exp_fields(arena[pl.ds(pl.multiple_of(r0, 8), 128), :])
            mx = jnp.max(jnp.maximum(hi, lo), axis=0, keepdims=True)
            mx = jnp.max(jnp.broadcast_to(mx, (8, Dh)), axis=1, keepdims=True)
            return _lsr(pltpu.bitcast(jnp.broadcast_to(mx, (8, Dh)), i32), 23)

        def pack_rows(r0, p0, emax, nb):
            r0 = pl.multiple_of(r0, 8)
            p0 = pl.multiple_of(p0, 8)
            width = 1 << nb
            base = jnp.clip(emax + (nb - 3) - (width - 1), 0, 256 - width)
            base7 = base * (128 * 65537)
            bad = jnp.zeros((8, Dh), i32)
            for g in range(NG):
                W = [arena[pl.ds(r0 + (g * 16 + i) * 8, 8), :] for i in range(16)]
                P, b = _encode(W, base7, nb)
                bad = bad | b
                for i in range(8 + nb):
                    arena[pl.ds(p0 + (g * (8 + nb) + i) * 8, 8), :] = P[i]
            return base, bad

        def softmax_step(qb, kmat):
            s = lax.dot_general(qb, kmat, (((1,), (1,)), ((), ())), preferred_element_type=f32)
            s = s * qk_scale
            m = st[0]
            m_new = jnp.maximum(m, jnp.max(s, axis=1, keepdims=True))
            alpha = jnp.exp2(m - m_new)
            p = jnp.exp2(s - m_new[:, 0:1])
            st[0] = m_new
            st[1] = alpha * st[1] + jnp.sum(p, axis=1, keepdims=True)
            return alpha, p.astype(bf16)

        def pv_step(alpha, pb, vmat):
            st[2] = alpha * st[2] + jnp.dot(pb, vmat, preferred_element_type=f32)

        def attention(xn, layer):
            xn8 = jnp.broadcast_to(xn, (QR, D)).astype(bf16)

            def head_body(hi, out_acc):
                h = hi if layer == 0 else Hkv - 1 - hi
                if layer == 0:
                    wait(head_w_copies(h, layer, 0))
                else:
                    pl.when(h < NW)(lambda: wait(head_w_copies(h, layer, 0)))
                q = None
                for g in range(G):
                    qg = jnp.dot(xn8, head_w(h, layer, 0, g), preferred_element_type=f32)
                    q = qg if q is None else jnp.where(row == g, qg, q)
                qb = q.astype(bf16)
                st[0] = jnp.full((QR, Dh), -jnp.inf, f32)
                st[1] = jnp.zeros((QR, Dh), f32)
                st[2] = jnp.zeros((QR, Dh), f32)

                def unit_first(ji, carry):
                    c = h * UPH + ji
                    r0 = SB + (c % NST) * 2 * RW
                    kc, vc = stage_copies(c)
                    kc.wait()
                    alpha, pb = softmax_step(qb, raw_rows(r0))
                    kemax = sample_emax(r0)
                    vc.wait()
                    pv_step(alpha, pb, raw_rows(r0 + RW))
                    vemax = sample_emax(r0 + RW)

                    @pl.when(c < NSMIN)
                    def _():
                        mx, mn = st[3], st[4]
                        for rr in (r0, r0 + RW):
                            for i in range(16):
                                hi_, lo_ = _exp_fields(arena[pl.ds(pl.multiple_of(rr + 8 * i, 8), 8), :])
                                mx = jnp.maximum(mx, jnp.maximum(hi_, lo_))
                                mn = jnp.minimum(mn, jnp.minimum(hi_, lo_))
                        st[3] = mx
                        st[4] = mn

                        @pl.when(c == NSMIN - 1)
                        def _():
                            narrow = jnp.max(mx) <= jnp.min(mn) * 8192.0
                            if _FORCE is None:
                                cfg[0] = jnp.where(narrow, 4, 5)
                            else:
                                cfg[0] = _FORCE

                    def keep(nb):
                        @pl.when((c >= NSS[nb]) & (c < C - NST))
                        def _():
                            z = C - NST - 1 - c
                            pw = PWS[nb]
                            kbase, kbad = pack_rows(r0, z * 2 * pw, kemax, nb)
                            vbase, vbad = pack_rows(r0 + RW, z * 2 * pw + pw, vemax, nb)
                            meta[0, z] = kbase[0, 0]
                            meta[1, z] = vbase[0, 0]
                            lossy = ((kbad | vbad) & _M_BAD[nb]) != 0
                            meta[2, z] = jnp.max(jnp.where(lossy, 1.0, 0.0)).astype(i32)

                    by_format(keep)

                    @pl.when(c + NST < C)
                    def _():
                        start(stage_copies(c + NST))

                    @pl.when(c + NST == C - 1)
                    def _():
                        w2_cp.start()

                        start(head_w_copies(NW - 1, 1, 0))
                    return carry

                def unit_second(ji, carry):
                    c = h * UPH + (UPH - 1 - ji)
                    ns = n_streamed()
                    packed = (c >= ns) & (c < C - NST)
                    z = jnp.clip(C - NST - 1 - c, 0, ZMAX - 1)

                    @pl.when(jnp.logical_not(packed))
                    def _():
                        j = 2 * jnp.maximum(ns - 1 - c, 0)
                        streamed = c < ns
                        r0 = SB + (c % NST) * 2 * RW
                        e = 2 * (C - 1 - c)

                        @pl.when(streamed)
                        def _():
                            half_copy(j, ns, k32).wait()
                        alpha, pb = softmax_step(qb, raw_rows(jnp.where(streamed, slot_row(NW + j), r0)))

                        @pl.when(streamed)
                        def _():
                            half_copy(j + 1, ns, v32).wait()

                        @pl.when(jnp.logical_not(streamed))
                        def _():
                            refill(e + 1, ns)
                        pv_step(alpha, pb, raw_rows(jnp.where(streamed, slot_row(NW + j + 1), r0 + RW)))

                        @pl.when(jnp.logical_not(streamed))
                        def _():
                            refill(e + 2, ns)

                    @pl.when(packed)
                    def _():
                        lossless = meta[2, z] == 0
                        pw = jnp.where(cfg[0] == 4, PWS[4], PWS[5])

                        def unpack_attend(nb):
                            @pl.when(lossless)
                            def _():
                                p0 = z * 2 * PWS[nb]
                                alpha, pb = softmax_step(qb, unpack_rows(p0, meta[0, z], nb))
                                pv_step(alpha, pb, unpack_rows(p0 + PWS[nb], meta[1, z], nb))

                        by_format(unpack_attend)

                        @pl.when(jnp.logical_not(lossless))
                        def _():
                            r = pl.multiple_of((c % UPH) * RW, RW)
                            p0 = pl.multiple_of(z * 2 * pw, 8)
                            zone = arena.at[pl.ds(p0, RW)]
                            kc = pltpu.make_async_copy(k32.at[0, h, pl.ds(r, RW)], zone, fsem.at[0])
                            kc.start()
                            kc.wait()
                            alpha, pb = softmax_step(qb, raw_rows(p0))
                            vc = pltpu.make_async_copy(v32.at[0, h, pl.ds(r, RW)], zone, fsem.at[0])
                            vc.start()
                            vc.wait()
                            pv_step(alpha, pb, raw_rows(p0))

                        refill(2 * (C - 1 - c) + 1, ns)
                        refill(2 * (C - 1 - c) + 2, ns)
                    return carry

                lax.fori_loop(0, UPH, unit_first if layer == 0 else unit_second, 0)
                o = (st[2] / st[1]).astype(bf16)
                zero = jnp.zeros_like(o)
                od = jnp.concatenate([jnp.where(row == g, o, zero) for g in range(G)], axis=1)
                if layer == 0:
                    wait(head_w_copies(h, layer, 1))
                else:
                    pl.when(h < NW)(lambda: wait(head_w_copies(h, layer, 1)))
                y = jnp.concatenate(
                    [jnp.dot(od, head_w(h, layer, 1, g), preferred_element_type=f32) for g in range(G)], axis=1)
                if layer == 0:
                    @pl.when(h + 2 < NW)
                    def _():
                        start(head_w_copies(h + 2, 0, 0))
                        start(head_w_copies(h + 2, 0, 1))
                return out_acc + y

            out = lax.fori_loop(0, Hkv, head_body, jnp.zeros((QR, D), f32))
            return jnp.sum(out, axis=0, keepdims=True)

        def mlp(xn, pending):
            xn8 = jnp.broadcast_to(xn, (QR, D)).astype(bf16)
            hmid = jnp.dot(xn8, w1[...], preferred_element_type=f32) + b1b[...].astype(f32).reshape(1, F)
            sp = jnp.log1p(jnp.exp(-jnp.abs(hmid))) + jnp.maximum(hmid, 0.0)
            act = hmid * jnp.tanh(sp)
            if pending is not None:
                pending.wait()
            y = jnp.dot(act.astype(bf16), w2[...], preferred_element_type=f32)
            return y[0:1, :]

        def rnd(t):
            return t.astype(bf16).astype(f32)

        x_cp.wait()
        x = xb[0].astype(f32)
        for layer in range(2):
            x = rnd(x + rnd(attention(_layernorm(x), layer)))
            if layer == 0:
                w1_cp.wait()
                b1_cp.wait()
            x = rnd(x + rnd(mlp(_layernorm(x), w2_cp if layer == 0 else None)))
        o_ref[0] = x.astype(o_ref.dtype)

    hbm = pl.BlockSpec(memory_space=pl.ANY)
    return pl.pallas_call(
        kernel,
        out_shape=jax.ShapeDtypeStruct(A_x.shape, A_x.dtype),
        in_specs=[hbm] * 8,
        out_specs=pl.BlockSpec(memory_space=pltpu.VMEM),
        scratch_shapes=[
            pltpu.VMEM((ROWS, Dh), i32),
            pltpu.VMEM((D, F), bf16),
            pltpu.VMEM((F, D), bf16),
            pltpu.VMEM(A_x.shape, bf16),
            pltpu.VMEM((F,), bf16),
            pltpu.VMEM((5, QR, Dh), f32),
            pltpu.SMEM((3, ZMAX), i32),
            pltpu.SMEM((1,), i32),
            pltpu.SemaphoreType.DMA((NSMAX,)),
            pltpu.SemaphoreType.DMA((NSMAX,)),
            pltpu.SemaphoreType.DMA((2, Hkv)),
            pltpu.SemaphoreType.DMA((4,)),
            pltpu.SemaphoreType.DMA((1,)),
        ],
        compiler_params=pltpu.CompilerParams(vmem_limit_bytes=128 * 1024 * 1024),
    )(A_x, A_k_cache, A_v_cache, A_wq, A_wo, B_w1, B_b1, B_w2)
```

```python
import math

import numpy as np
import jax
import jax.numpy as jnp
from jax import lax
import jax.experimental.pallas as pl
import jax.experimental.pallas.tpu as pltpu

_BS = 4096
_NSTAGE = 2
_PACK_ROWS = 243968
_NH = 2
_EPS = 1e-5


def _c32(v):
    return np.uint32(v).astype(np.int32)


_M_E = _c32(0x7F807F80)
_M_SM = _c32(0x807F807F)
_M_M = _c32(0x007F007F)
_M_M7 = _c32(0x3F803F80)
_M_S14 = _c32(0x40004000)
_M_S15 = _c32(0x80008000)
_M_D = {4: _c32(0x07800780), 5: _c32(0x0F800F80)}
_M_BAD = {4: _c32(0xF800F800), 5: _c32(0xF000F000)}


def _lsr(x, n):
    return lax.shift_right_logical(x, jnp.int32(n))


def _lsl(x, n):
    return lax.shift_left(x, jnp.int32(n))


def _encode(W, base7, nb):
    out = []
    for j in range(8):
        a, b = W[2 * j], W[2 * j + 1]
        out.append((a & _M_SM) | (_lsl(b, 7) & _M_M7) | (_lsr(b, 1) & _M_S14))
    t = [(w & _M_E) - base7 for w in W]
    bad = t[0]
    for w in t[1:]:
        bad = bad | w
    if nb == 5:
        for i in range(5):
            out.append(_lsr(t[3 * i], 7) | _lsr(t[3 * i + 1], 2) | _lsl(t[3 * i + 2], 3)
                       | (_lsl(t[15], 8 - i) & _M_S15))
    else:
        for i in range(4):
            out.append(_lsr(t[4 * i], 7) | _lsr(t[4 * i + 1], 3) | _lsl(t[4 * i + 2], 1) | _lsl(t[4 * i + 3], 5))
    return out, bad


def _decode(P, base7, nb):
    S, E = P[:8], P[8:]
    W = [None] * 16
    for j in range(8):
        W[2 * j] = S[j] & _M_SM
        W[2 * j + 1] = (_lsr(S[j], 7) & _M_M) | (_lsl(S[j], 1) & _M_S15)
    m = _M_D[nb]
    if nb == 5:
        for i in range(5):
            W[3 * i] = W[3 * i] | ((_lsl(E[i], 7) & m) + base7)
            W[3 * i + 1] = W[3 * i + 1] | ((_lsl(E[i], 2) & m) + base7)
            W[3 * i + 2] = W[3 * i + 2] | ((_lsr(E[i], 3) & m) + base7)
        d = None
        for i in range(5):
            b = _lsr(E[i], 8 - i) & _c32(0x00800080 << i)
            d = b if d is None else d | b
        W[15] = W[15] | (d + base7)
    else:
        for i in range(4):
            W[4 * i] = W[4 * i] | ((_lsl(E[i], 7) & m) + base7)
            W[4 * i + 1] = W[4 * i + 1] | ((_lsl(E[i], 3) & m) + base7)
            W[4 * i + 2] = W[4 * i + 2] | ((_lsr(E[i], 1) & m) + base7)
            W[4 * i + 3] = W[4 * i + 3] | ((_lsr(E[i], 5) & m) + base7)
    return W


def _exp_fields(w):
    hi = pltpu.bitcast(w & _c32(0x7F800000), jnp.float32)
    lo = pltpu.bitcast(_lsl(w, 16) & _c32(0x7F800000), jnp.float32)
    return hi, lo


def _layernorm(x):
    m = jnp.mean(x, axis=-1, keepdims=True)
    d = x - m
    v = jnp.mean(d * d, axis=-1, keepdims=True)
    return d / jnp.sqrt(v + _EPS)


@jax.jit
def pallas_interleave_layers__gqa_block_cached__dense_activation_mish__decode_kernel(
    A_x: jax.Array,
    A_k_cache: jax.Array,
    A_v_cache: jax.Array,
    A_wq: jax.Array,
    A_wo: jax.Array,
    B_x: jax.Array,
    B_w1: jax.Array,
    B_b1: jax.Array,
    B_w2: jax.Array,
):
    del B_x
    _, _, D = A_x.shape
    _, Hkv, S, Dh = A_k_cache.shape
    Hq = A_wq.shape[1] // Dh
    G = Hq // Hkv
    GD = G * Dh
    F = B_w1.shape[1]
    BS, NST = _BS, _NSTAGE
    RW = BS // 2
    NG = RW // 128
    PWS = {nb: NG * 8 * (8 + nb) for nb in (4, 5)}
    UPH = S // BS
    C = Hkv * UPH
    SB = _PACK_ROWS
    HW = D // 2
    WB = SB + NST * 2 * RW
    ROWS = WB + 2 * G * HW
    NW = Hkv - 1
    ZS = {nb: SB // (2 * PWS[nb]) for nb in (4, 5)}
    NSS = {nb: C - NST - ZS[nb] for nb in (4, 5)}
    ZMAX, NSMAX, NSMIN = max(ZS.values()), max(NSS.values()), min(NSS.values())
    for nb in (4, 5):
        assert NSS[nb] >= NST and (NW + 2 * NSS[nb] - 2 * NST) * RW <= ZS[nb] * 2 * PWS[nb]
        assert ZS[nb] * 2 * PWS[nb] + G * HW <= SB
    assert 2 * G * HW == RW and GD == D
    assert C % NST == 0
    NGRP = 3 + (NSMAX - 1) // 8 + 2
    NH = _NH
    QR = 8
    qk_scale = (Dh ** -0.5) * math.log2(math.e)
    bf16, f32, i32 = jnp.bfloat16, jnp.float32, jnp.int32

    def kernel(x_hbm, k_hbm, v_hbm, wq_hbm, wo_hbm, w1_hbm, b1_hbm, w2_hbm, o_ref,
               arena, w1, w2, xb, b1b, st, meta, cfg, ksem, vsem, gsem, hsem, wsem, fsem):
        k32 = k_hbm.bitcast(i32)
        v32 = v_hbm.bitcast(i32)
        wq32 = wq_hbm.bitcast(i32)
        wo32 = wo_hbm.bitcast(i32)

        def kv_copies(c, row, si):
            h = c // UPH
            r = pl.multiple_of((c % UPH) * RW, RW)
            row = pl.multiple_of(row, 8)
            return (pltpu.make_async_copy(k32.at[0, h, pl.ds(r, RW)], arena.at[pl.ds(row, RW)], ksem.at[si]),
                    pltpu.make_async_copy(v32.at[0, h, pl.ds(r, RW)], arena.at[pl.ds(row + RW, RW)], vsem.at[si]))

        def stage_copies(c):
            s = c % NST
            return kv_copies(c, SB + s * 2 * RW, s)

        def slot_row(s):
            stage = SB + ((NST - 1 - s // 2) * 2 + s % 2) * RW
            return jnp.where(s < 2 * NST, stage, (s - 2 * NST) * RW)

        def slots_free(e):
            pw = jnp.where(cfg[0] == 4, PWS[4], PWS[5])
            return jnp.minimum(e, 2 * NST) + (jnp.maximum(e - 2 * NST, 0) * pw) // RW

        def half_copy(j, ns, src):
            c = ns - 1 - j // 2
            h = c // UPH
            r = pl.multiple_of((c % UPH) * RW, RW)
            row = pl.multiple_of(slot_row(NW + j), 8)
            grp = jnp.where(c < 8, sum((c >= (1 << b)).astype(i32) for b in range(3)), 3 + c // 8)
            sem = gsem.at[grp if src is k32 else jnp.where(c == 0, NGRP - 1, grp)]
            return pltpu.make_async_copy(src.at[0, h, pl.ds(r, RW)], arena.at[pl.ds(row, RW)], sem)

        def head_w_row(h, layer, is_o):
            if layer == 0:
                r = (h % 2) * RW
            else:
                r = slot_row(NW - 1 - h)
            r = r + is_o * G * HW
            if layer == 1 and not is_o:
                spare = jnp.where(cfg[0] == 4, ZS[4] * 2 * PWS[4], ZS[5] * 2 * PWS[5])
                r = jnp.where(h == NW - 1, spare, r)
            return jnp.where(h == NW, WB + is_o * G * HW, r)

        def head_w_copies(h, layer, is_o):
            row = pl.multiple_of(head_w_row(h, layer, is_o), 8)
            cps = []
            for g in range(G):
                if is_o:
                    src = wo32.at[pl.ds(pl.multiple_of(h * G * Dh // 2, HW), HW), pl.ds(g * Dh, Dh)]
                else:
                    src = wq32.at[:, pl.ds(pl.multiple_of(h * GD + g * Dh, Dh), Dh)]
                cps.append(pltpu.make_async_copy(src, arena.at[pl.ds(row + g * HW, HW)], hsem.at[h]))
            return cps

        def head_w(h, layer, is_o, g):
            row = pl.multiple_of(head_w_row(h, layer, is_o) + g * HW, 8)
            return pltpu.bitcast(arena[pl.ds(row, HW), :], bf16)

        def refill(e, ns):
            s = slots_free(e) - 1
            fresh = s >= slots_free(e - 1)
            j = s - NW

            @pl.when(fresh & (s < NW))
            def _():
                @pl.when(s > 0)
                def _():
                    start(head_w_copies(NW - 1 - s, 1, 0))
                start(head_w_copies(NW - 1 - s, 1, 1))

            @pl.when(fresh & (j >= 0) & (j < 2 * ns))
            def _():
                @pl.when(j % 2 == 0)
                def _():
                    half_copy(j, ns, k32).start()

                @pl.when(j % 2 == 1)
                def _():
                    half_copy(j, ns, v32).start()

        def start(cps):
            for cp in cps:
                cp.start()

        def wait(cps):
            for cp in cps:
                cp.wait()

        x_cp = pltpu.make_async_copy(x_hbm, xb, wsem.at[0])
        w1_cp = pltpu.make_async_copy(w1_hbm, w1, wsem.at[1])
        b1_cp = pltpu.make_async_copy(b1_hbm, b1b, wsem.at[2])
        w2_cp = pltpu.make_async_copy(w2_hbm, w2, wsem.at[3])
        for c in range(NST):
            start(stage_copies(c))
        x_cp.start()
        start(head_w_copies(0, 0, 0))
        start(head_w_copies(0, 0, 1))
        for is_o in (0, 1):
            start(head_w_copies(1, 0, is_o))
            start(head_w_copies(NW, 0, is_o))
        w1_cp.start()
        b1_cp.start()

        cfg[0] = 5
        st[3] = jnp.zeros((QR, Dh), f32)
        st[4] = jnp.full((QR, Dh), jnp.inf, f32)
        row = lax.broadcasted_iota(i32, (QR, Dh), 0)

        def by_format(fn):
            for nb in (4, 5):
                pl.when(cfg[0] == nb)(lambda nb=nb: fn(nb))

        def n_streamed():
            return jnp.where(cfg[0] == 4, NSS[4], NSS[5])

        def raw_rows(r0):
            return pltpu.bitcast(arena[pl.ds(pl.multiple_of(r0, 8), RW), :], bf16)

        def unpack_rows(p0, base, nb, blk):
            p0 = pl.multiple_of(p0, 8)
            base7 = jnp.full((8, Dh), base * (128 * 65537), i32)
            words = []
            for g in range(blk * NG // NH, (blk + 1) * NG // NH):
                P = [arena[pl.ds(p0 + (g * (8 + nb) + i) * 8, 8), :] for i in range(8 + nb)]
                words += _decode(P, base7, nb)
            return pltpu.bitcast(jnp.concatenate(words, axis=0), bf16)

        def sample_emax(r0):
            hi, lo = _exp_fields(arena[pl.ds(pl.multiple_of(r0, 8), 128), :])
            mx = jnp.max(jnp.maximum(hi, lo), axis=0, keepdims=True)
            mx = jnp.max(jnp.broadcast_to(mx, (8, Dh)), axis=1, keepdims=True)
            return _lsr(pltpu.bitcast(jnp.broadcast_to(mx, (8, Dh)), i32), 23)

        def pack_rows(r0, p0, emax, nb):
            r0 = pl.multiple_of(r0, 8)
            p0 = pl.multiple_of(p0, 8)
            width = 1 << nb
            base = jnp.clip(emax + (nb - 3) - (width - 1), 0, 256 - width)
            base7 = base * (128 * 65537)
            bad = jnp.zeros((8, Dh), i32)
            for g in range(NG):
                W = [arena[pl.ds(r0 + (g * 16 + i) * 8, 8), :] for i in range(16)]
                P, b = _encode(W, base7, nb)
                bad = bad | b
                for i in range(8 + nb):
                    arena[pl.ds(p0 + (g * (8 + nb) + i) * 8, 8), :] = P[i]
            return base, bad

        def softmax_step(qb, kmat):
            s = lax.dot_general(qb, kmat, (((1,), (1,)), ((), ())), preferred_element_type=f32)
            s = s * qk_scale
            m = st[0]
            m_new = jnp.maximum(m, jnp.max(s, axis=1, keepdims=True))
            alpha = jnp.exp2(m - m_new)
            p = jnp.exp2(s - m_new[:, 0:1])
            st[0] = m_new
            st[1] = alpha * st[1] + jnp.sum(p, axis=1, keepdims=True)
            return alpha, p.astype(bf16)

        def pv_step(alpha, pb, vmat):
            st[2] = alpha * st[2] + jnp.dot(pb, vmat, preferred_element_type=f32)

        def attend_packed(qb, p0, kbase, vbase, nb):
            m, l, acc = st[0], st[1], st[2]
            ss = [lax.dot_general(qb, unpack_rows(p0, kbase, nb, b), (((1,), (1,)), ((), ())),
                                  preferred_element_type=f32) * qk_scale for b in range(NH)]
            for b, s in enumerate(ss):
                m_new = jnp.maximum(m, jnp.max(s, axis=1, keepdims=True))
                alpha = jnp.exp2(m - m_new)
                p = jnp.exp2(s - m_new[:, 0:1])
                l = alpha * l + jnp.sum(p, axis=1, keepdims=True)
                acc = alpha * acc + jnp.dot(p.astype(bf16), unpack_rows(p0 + PWS[nb], vbase, nb, b),
                                            preferred_element_type=f32)
                m = m_new
            st[0], st[1], st[2] = m, l, acc

        def attention(xn, layer):
            xn8 = jnp.broadcast_to(xn, (QR, D)).astype(bf16)

            def head_body(hi, out_acc):
                h = hi if layer == 0 else Hkv - 1 - hi
                if layer == 0:
                    wait(head_w_copies(h, layer, 0) + head_w_copies(h, layer, 1))
                else:
                    pl.when(h < NW)(lambda: wait(head_w_copies(h, layer, 0) + head_w_copies(h, layer, 1)))
                q = None
                for g in range(G):
                    qg = jnp.dot(xn8, head_w(h, layer, 0, g), preferred_element_type=f32)
                    q = qg if q is None else jnp.where(row == g, qg, q)
                qb = q.astype(bf16)
                st[0] = jnp.full((QR, Dh), -jnp.inf, f32)
                st[1] = jnp.zeros((QR, Dh), f32)
                st[2] = jnp.zeros((QR, Dh), f32)

                def unit_first(ji, carry):
                    c = h * UPH + ji
                    r0 = SB + (c % NST) * 2 * RW
                    kc, vc = stage_copies(c)
                    kc.wait()
                    alpha, pb = softmax_step(qb, raw_rows(r0))
                    kemax = sample_emax(r0)
                    vc.wait()
                    pl.when(c == C - 1)(lambda: start(head_w_copies(NW - 1, 1, 0)))
                    pv_step(alpha, pb, raw_rows(r0 + RW))
                    vemax = sample_emax(r0 + RW)

                    @pl.when(c < NSMIN)
                    def _():
                        mx, mn = st[3], st[4]
                        for rr in (r0, r0 + RW):
                            for i in range(16):
                                hi_, lo_ = _exp_fields(arena[pl.ds(pl.multiple_of(rr + 8 * i, 8), 8), :])
                                mx = jnp.maximum(mx, jnp.maximum(hi_, lo_))
                                mn = jnp.minimum(mn, jnp.minimum(hi_, lo_))
                        st[3] = mx
                        st[4] = mn

                        @pl.when(c == NSMIN - 1)
                        def _():
                            narrow = jnp.max(mx) <= jnp.min(mn) * 8192.0
                            cfg[0] = jnp.where(narrow, 4, 5)

                    def keep(nb):
                        @pl.when((c >= NSS[nb]) & (c < C - NST))
                        def _():
                            z = C - NST - 1 - c
                            pw = PWS[nb]
                            kbase, kbad = pack_rows(r0, z * 2 * pw, kemax, nb)
                            vbase, vbad = pack_rows(r0 + RW, z * 2 * pw + pw, vemax, nb)
                            meta[0, z] = kbase[0, 0]
                            meta[1, z] = vbase[0, 0]
                            lossy = ((kbad | vbad) & _M_BAD[nb]) != 0
                            meta[2, z] = jnp.max(jnp.where(lossy, 1.0, 0.0)).astype(i32)

                    by_format(keep)

                    @pl.when(c + NST < C)
                    def _():
                        start(stage_copies(c + NST))

                    @pl.when(c + NST == C - 1)
                    def _():
                        w2_cp.start()
                    return carry

                def unit_second(ji, carry):
                    c = h * UPH + (UPH - 1 - ji)
                    ns = n_streamed()
                    packed = (c >= ns) & (c < C - NST)
                    z = jnp.clip(C - NST - 1 - c, 0, ZMAX - 1)

                    @pl.when(jnp.logical_not(packed))
                    def _():
                        j = 2 * jnp.maximum(ns - 1 - c, 0)
                        streamed = c < ns
                        r0 = SB + (c % NST) * 2 * RW
                        e = 2 * (C - 1 - c)

                        top = (c == ns - 1) | (((c + 1) & c) == 0) | (c % 8 == 7)

                        @pl.when(streamed & (c > 0) & top)
                        def _():
                            lo = jnp.where(c < 8, 1 << sum((c >= (2 << b)).astype(i32) for b in range(2)), c - c % 8)

                            def group_wait(t, carry):
                                half_copy(2 * (ns - 1 - t), ns, k32).wait()
                                half_copy(2 * (ns - 1 - t) + 1, ns, v32).wait()
                                return carry

                            lax.fori_loop(lo, c + 1, group_wait, 0)

                        @pl.when(c == 0)
                        def _():
                            half_copy(j, ns, k32).wait()
                        alpha, pb = softmax_step(qb, raw_rows(jnp.where(streamed, slot_row(NW + j), r0)))

                        @pl.when(c == 0)
                        def _():
                            half_copy(j + 1, ns, v32).wait()

                        @pl.when(jnp.logical_not(streamed))
                        def _():
                            refill(e + 1, ns)
                        pv_step(alpha, pb, raw_rows(jnp.where(streamed, slot_row(NW + j + 1), r0 + RW)))

                        @pl.when(jnp.logical_not(streamed))
                        def _():
                            refill(e + 2, ns)

                    @pl.when(packed)
                    def _():
                        lossless = meta[2, z] == 0
                        pw = jnp.where(cfg[0] == 4, PWS[4], PWS[5])

                        def unpack_attend(nb):
                            @pl.when(lossless)
                            def _():
                                attend_packed(qb, z * 2 * PWS[nb], meta[0, z], meta[1, z], nb)

                        by_format(unpack_attend)

                        @pl.when(jnp.logical_not(lossless))
                        def _():
                            r = pl.multiple_of((c % UPH) * RW, RW)
                            p0 = pl.multiple_of(z * 2 * pw, 8)
                            zone = arena.at[pl.ds(p0, RW)]
                            kc = pltpu.make_async_copy(k32.at[0, h, pl.ds(r, RW)], zone, fsem.at[0])
                            kc.start()
                            kc.wait()
                            alpha, pb = softmax_step(qb, raw_rows(p0))
                            vc = pltpu.make_async_copy(v32.at[0, h, pl.ds(r, RW)], zone, fsem.at[0])
                            vc.start()
                            vc.wait()
                            pv_step(alpha, pb, raw_rows(p0))

                        refill(2 * (C - 1 - c) + 1, ns)
                        refill(2 * (C - 1 - c) + 2, ns)
                    return carry

                lax.fori_loop(0, UPH, unit_first if layer == 0 else unit_second, 0)
                o = (st[2] / st[1]).astype(bf16)
                zero = jnp.zeros_like(o)
                od = jnp.concatenate([jnp.where(row == g, o, zero) for g in range(G)], axis=1)
                y = jnp.concatenate(
                    [jnp.dot(od, head_w(h, layer, 1, g), preferred_element_type=f32) for g in range(G)], axis=1)
                if layer == 0:
                    @pl.when(h + 2 < NW)
                    def _():
                        start(head_w_copies(h + 2, 0, 0))
                        start(head_w_copies(h + 2, 0, 1))
                return out_acc + y

            out = lax.fori_loop(0, Hkv, head_body, jnp.zeros((QR, D), f32))
            return jnp.sum(out, axis=0, keepdims=True)

        def mlp(xn, pending):
            xn8 = jnp.broadcast_to(xn, (QR, D)).astype(bf16)
            hmid = jnp.dot(xn8, w1[...], preferred_element_type=f32) + b1b[...].astype(f32).reshape(1, F)
            sp = jnp.log1p(jnp.exp(-jnp.abs(hmid))) + jnp.maximum(hmid, 0.0)
            act = hmid * jnp.tanh(sp)
            if pending is not None:
                pending.wait()
            y = jnp.dot(act.astype(bf16), w2[...], preferred_element_type=f32)
            return y[0:1, :]

        def rnd(t):
            return t.astype(bf16).astype(f32)

        x_cp.wait()
        x = xb[0].astype(f32)
        for layer in range(2):
            x = rnd(x + rnd(attention(_layernorm(x), layer)))
            if layer == 0:
                w1_cp.wait()
                b1_cp.wait()
            x = rnd(x + rnd(mlp(_layernorm(x), w2_cp if layer == 0 else None)))
        o_ref[0] = x.astype(o_ref.dtype)

    hbm = pl.BlockSpec(memory_space=pl.ANY)
    return pl.pallas_call(
        kernel,
        out_shape=jax.ShapeDtypeStruct(A_x.shape, A_x.dtype),
        in_specs=[hbm] * 8,
        out_specs=pl.BlockSpec(memory_space=pltpu.VMEM),
        scratch_shapes=[
            pltpu.VMEM((ROWS, Dh), i32),
            pltpu.VMEM((D, F), bf16),
            pltpu.VMEM((F, D), bf16),
            pltpu.VMEM(A_x.shape, bf16),
            pltpu.VMEM((F,), bf16),
            pltpu.VMEM((5, QR, Dh), f32),
            pltpu.SMEM((3, ZMAX), i32),
            pltpu.SMEM((1,), i32),
            pltpu.SemaphoreType.DMA((NST,)),
            pltpu.SemaphoreType.DMA((NST,)),
            pltpu.SemaphoreType.DMA((NGRP,)),
            pltpu.SemaphoreType.DMA((Hkv,)),
            pltpu.SemaphoreType.DMA((4,)),
            pltpu.SemaphoreType.DMA((1,)),
        ],
        compiler_params=pltpu.CompilerParams(vmem_limit_bytes=128 * 1024 * 1024),
    )(A_x, A_k_cache, A_v_cache, A_wq, A_wo, B_w1, B_b1, B_w2)
```
